```python
import jax
import jax.numpy as jnp

def _softmax(x, axis=-1):
    return jax.nn.softmax(x, axis=axis)
def _gelu(x):
    return jax.nn.gelu(x, approximate=True)
def _silu(x):
    return jax.nn.silu(x)
def _sigmoid(x):
    return jax.nn.sigmoid(x)
def _layernorm(x, axis=-1, eps=1e-5):
    m = jnp.mean(x, axis=axis, keepdims=True)
    v = jnp.var(x, axis=axis, keepdims=True)
    return (x - m) / jnp.sqrt(v + eps)
def _scatter_add(tgt, idx, src, axis=0):
    return tgt.at[idx].add(src)
def _segment_sum(src, seg, n):
    return jax.ops.segment_sum(src, seg, n)
class _Rng:
    def __init__(self, key):
        self._k = key
    def _next(self):
        self._k, sub = jax.random.split(self._k)
        return sub
    def normal(self, shape):
        return jax.random.normal(self._next(), shape, dtype=jnp.bfloat16)
    def randint(self, lo, hi, shape):
        return jax.random.randint(self._next(), shape, lo, hi, dtype=jnp.int32)
    def uniform(self, shape, lo=0.0, hi=1.0):
        return jax.random.uniform(self._next(), shape, jnp.bfloat16, lo, hi)
    def permutation(self, n):
        return jax.random.permutation(self._next(), n)


kernel_name = 'interleave_layers__ssm_conv_h3__mixer_s_mlp__prompt'

def setup_inputs():
    _rng = _Rng(jax.random.key(int.from_bytes(__import__("os").urandom(4), "little")))
    _w = (lambda a: (lambda t: t.astype(jnp.bfloat16) if jnp.issubdtype(t.dtype, jnp.floating) else t)(jnp.asarray(a)))
    def _A_setup():
        B, S, D = 1, 2048, 1024
        ks = 4
        return {
            "q": _w((lambda *s: _rng.normal(s) * 0.05)(B, S, D)),
            "k": _w((lambda *s: _rng.normal(s) * 0.05)(B, S, D)),
            "v": _w((lambda *s: _rng.normal(s) * 0.05)(B, S, D)),
            "shift_k": _w((lambda *s: _rng.normal(s) * 0.05)(D, ks) * 0.5),
            "ssm_k": _w((lambda *s: _rng.normal(s) * 0.05)(D, S) * (1.0 / S ** 0.5)),
            "ssm_D": _w((lambda *s: _rng.normal(s) * 0.05)(D)),
        }
    _A_in = _A_setup()

    def _B_setup():
        B, S, D, F = 1, 2048, 1024, 3584
        return {
            "x":  _w((lambda *s: _rng.normal(s) * 0.05)(B, S, D)),
            "w1": _w((lambda *s: _rng.normal(s) * 0.05)(D, D) * (D ** -0.5)),
            "w2": _w((lambda *s: _rng.normal(s) * 0.05)(D, D) * (D ** -0.5)),
            "w3": _w((lambda *s: _rng.normal(s) * 0.05)(D, F) * (D ** -0.5)),
            "w4": _w((lambda *s: _rng.normal(s) * 0.05)(F, D) * (F ** -0.5)),
        }
    _B_in = _B_setup()

    return {
        "A_q": _A_in["q"],
        "A_k": _A_in["k"],
        "A_v": _A_in["v"],
        "A_shift_k": _A_in["shift_k"],
        "A_ssm_k": _A_in["ssm_k"],
        "A_ssm_D": _A_in["ssm_D"],
        "B_x": _B_in["x"],
        "B_w1": _B_in["w1"],
        "B_w2": _B_in["w2"],
        "B_w3": _B_in["w3"],
        "B_w4": _B_in["w4"],
    }

def reference(A_q, A_k, A_v, A_shift_k, A_ssm_k, A_ssm_D, B_x, B_w1, B_w2, B_w3, B_w4):
    def _A_ref(q, k, v, shift_k, ssm_k, ssm_D):
        B, S, D = q.shape
        ks = shift_k.shape[-1]
        k_pad = jnp.pad(k, ((0, 0), (ks - 1, 0), (0, 0)))
        k_shift = jnp.zeros_like(k)
        for t in range(ks):
            k_shift = k_shift + k_pad[:, t:t + S, :] * shift_k[:, ks - 1 - t][None, None, :]
        kv = k_shift * v
        L = 2 * S
        kv_pad = jnp.pad(kv, ((0, 0), (0, S), (0, 0)))
        kf_pad = jnp.pad(ssm_k, ((0, 0), (0, S)))
        kv_f = (lambda x, axes=(-2,-1): jnp.fft.rfft2(x.astype(jnp.float32), axes=axes))(kv_pad[:, None, :, :], axes=(1, 2))
        kf_f = (lambda x, axes=(-2,-1): jnp.fft.rfft2(x.astype(jnp.float32), axes=axes))(kf_pad[:, None, :], axes=(1, 2))
        kf_f = (lambda x, *d: x.transpose(*d))(kf_f, 1, 2, 0)
        y_f = kv_f * kf_f[None, :, :, :]
        y = (lambda x, s, axes=(-2,-1): jnp.fft.irfft2(x, s=s, axes=axes).astype(jnp.bfloat16))(y_f, (1, L), axes=(1, 2))[:, 0, :S, :]
        y = y + kv * ssm_D[None, None, :]
        return q * y

    def _B_ref(x, w1, w2, w3, w4):
        B, S, D = x.shape
        h = _gelu(_layernorm(x, axis=-1) @ w1)
        c = D // 4
        g0 = jnp.pad(h[:, :, 0*c:1*c], ((0, 0), (1, 0), (0, 0)))[:, :S, :]
        g1 = jnp.pad(h[:, :, 1*c:2*c], ((0, 0), (0, 1), (0, 0)))[:, 1:, :]
        g2 = jnp.pad(h[:, :, 2*c:3*c], ((0, 0), (2, 0), (0, 0)))[:, :S, :]
        g3 = jnp.pad(h[:, :, 3*c:   ], ((0, 0), (0, 2), (0, 0)))[:, 2:, :]
        hs = jnp.concatenate([g0, g1, g2, g3], axis=-1) @ w2
        x1 = x + hs
        h2 = _gelu(_layernorm(x1, axis=-1) @ w3) @ w4
        return x1 + h2

    x = A_q
    x = x + _A_ref(_layernorm(x, axis=-1), A_k, A_v, A_shift_k, A_ssm_k, A_ssm_D)
    x = x + _B_ref(_layernorm(x, axis=-1), B_w1, B_w2, B_w3, B_w4)
    x = x + _A_ref(_layernorm(x, axis=-1), A_k, A_v, A_shift_k, A_ssm_k, A_ssm_D)
    x = x + _B_ref(_layernorm(x, axis=-1), B_w1, B_w2, B_w3, B_w4)
    return x
```

```python
import numpy as np
import jax
import jax.numpy as jnp
from jax import lax
import jax.experimental.pallas as pl
import jax.experimental.pallas.tpu as pltpu

S, D, F = 2048, 1024, 3584
L = 128
NC = S // L
CB = 256
NCB = D // CB
TM = 512
NB = S // TM
FC = 896
EPS = 1e-5
RS = 32
NP = F // FC
PS = TM // NP
F32, BF16 = jnp.float32, jnp.bfloat16


def _dft_consts():
    f = np.arange(L)[:, None]
    j = np.arange(L)[None, :]
    ang = np.pi * (((4 * f + 1) * j) % (4 * L)) / (2 * L)
    fwd = np.concatenate([np.cos(ang), np.sin(ang)], axis=0)
    inv = np.concatenate([np.cos(ang).T, np.sin(ang).T], axis=1) / L
    return fwd.astype(jnp.bfloat16), inv.astype(jnp.bfloat16)


def _ln(x):
    m = jnp.mean(x, axis=-1, keepdims=True)
    c = x - m
    v = jnp.mean(c * c, axis=-1, keepdims=True)
    return c * lax.rsqrt(v + EPS)


def _gelu(x):
    c = 0.7978845608028654
    return 0.5 * x * (1.0 + jnp.tanh(c * (x + 0.044715 * (x * x * x))))


def _dot(a, b):
    return jnp.dot(a, b, preferred_element_type=F32)


def _kernel(q_hbm, k_hbm, v_hbm, sk_ref, ssm_hbm, sd_ref, w1_hbm, w2_hbm, w3_hbm, w4_hbm,
            fwd_ref, inv_ref, o_hbm,
            xbuf, qbuf, hb, ybuf, w1, w2, w3, w4, kb, vb, sb, SP0, zs, n2, nb0, nb1, hsf,
            sem_c, sem_w, sem_o):


    def conv_copies(cb, slot):
        return (
            pltpu.make_async_copy(k_hbm.at[0, :, pl.ds(cb * CB, CB)], kb.at[slot], sem_c.at[slot, 0]),
            pltpu.make_async_copy(v_hbm.at[0, :, pl.ds(cb * CB, CB)], vb.at[slot], sem_c.at[slot, 1]),
            pltpu.make_async_copy(ssm_hbm.at[pl.ds(cb * CB, CB), :], sb.at[slot], sem_c.at[slot, 2]),
        )

    def first_copies(h):
        r = pl.ds(h * (S // 2), S // 2)
        return (
            pltpu.make_async_copy(ssm_hbm.at[pl.ds(0, CB), r], sb.at[0, :, r], sem_c.at[h * NCB, 2]),
            pltpu.make_async_copy(k_hbm.at[0, r, pl.ds(0, CB)], kb.at[0, r, :], sem_c.at[h * NCB, 0]),
            pltpu.make_async_copy(v_hbm.at[0, r, pl.ds(0, CB)], vb.at[0, r, :], sem_c.at[h * NCB, 1]),
        )

    for c in first_copies(0):
        c.start()
    w_copies = [
        pltpu.make_async_copy(q_hbm.at[0], qbuf, sem_w.at[0]),
        pltpu.make_async_copy(w1_hbm, w1, sem_w.at[1]),
        pltpu.make_async_copy(w2_hbm, w2, sem_w.at[2]),
        pltpu.make_async_copy(w3_hbm, w3, sem_w.at[3]),
        pltpu.make_async_copy(w4_hbm, w4, sem_w.at[4]),
    ]

    taps = sk_ref[...].astype(F32)
    dskip = sd_ref[...].astype(F32).reshape(1, D)
    for l in range(2):
        hb[l, 0:8, :] = jnp.zeros((8, D), F32)
        hb[l, 8 + S:16 + S, :] = jnp.zeros((8, D), F32)
    zs[0] = 0
    z = zs[0]
    LT = CB // 128
    sp = SP0

    def lane(i):
        return slice(i * 128, (i + 1) * 128)

    def conv_in(cb):
        cs = slice(cb * CB, (cb + 1) * CB)
        tail = jnp.zeros((8, CB), F32)
        kprev = None
        for a in range(NC):
            r = slice(a * L, (a + 1) * L)
            if cb == 0 and a == NC // 2:
                for c in first_copies(1):
                    c.wait()
                for c in conv_copies(1, 1):
                    c.start()
            cur = kb[cb, r, :].astype(F32)
            win = jnp.concatenate([tail, cur], axis=0)
            tail = cur[L - 8:]
            ks = cur * taps[0:1, cs]
            for j in range(1, 4):
                ks = ks + pltpu.roll(win, j, 0)[8:] * taps[j:j + 1, cs]
            kv = ks * vb[cb, r, :].astype(F32)
            ybuf[r, cs] = kv * dskip[:, cs]
            um = _dot(fwd_ref[...], kv.astype(BF16))
            km = lax.dot_general(fwd_ref[...], sb[cb, :, r], (((1,), (1,)), ((), ())),
                                 preferred_element_type=F32)
            kr, ki = km[0:L], km[L:2 * L]
            if a:
                kr, ki = kr + kprev[L:2 * L], ki - kprev[0:L]
            kprev = km
            ur, ui = um[0:L], um[L:2 * L]
            for i, val in enumerate((ur + ui, ui, ur, kr, kr + ki, ki - kr)):
                for lt in range(LT):
                    sp[a, :, lane(6 * lt + i)] = val[:, lane(lt)]

    def spectra_product(t, _):
        rr = pl.ds(pl.multiple_of(t * 8, 8), 8)
        H = NC // 2
        for lt in range(LT):
            yr_l, yi_l = lane(6 * LT + 2 * lt), lane(6 * LT + 2 * lt + 1)
            for b0 in (0, H):
                u = [[sp[b, rr, lane(6 * lt + i)] for i in range(3)] for b in range(b0, b0 + H)]
                for a in range(b0, NC):
                    p = None
                    for b in range(b0, min(a, b0 + H - 1) + 1):
                        q = [u[b - b0][i] * sp[a - b, rr, lane(6 * lt + 3 + i)] for i in range(3)]
                        p = q if p is None else [p[i] + q[i] for i in range(3)]
                    yr, yi = p[0] - p[1], p[0] + p[2]
                    if b0:
                        yr, yi = yr + sp[a, rr, yr_l], yi + sp[a, rr, yi_l]
                    sp[a, rr, yr_l] = yr
                    sp[a, rr, yi_l] = yi
        return 0

    def conv_out(cb):
        for a in range(NC):
            yf = jnp.concatenate([
                jnp.concatenate([sp[a, :, lane(6 * LT + 2 * lt + i)] for lt in range(LT)], axis=1)
                for i in range(2)], axis=0)
            ybuf[a * L:(a + 1) * L, cb * CB:(cb + 1) * CB] += _dot(inv_ref[...], yf.astype(BF16))

    for cb in range(NCB):
        for c in (conv_copies(cb, cb) if cb else first_copies(0)):
            c.wait()
        if cb == 0:
            for c in first_copies(1):
                c.start()
        if 0 < cb < NCB - 1:
            for c in conv_copies(cb + 1, cb + 1):
                c.start()
        for c in (w_copies[0:0], w_copies[0:1], w_copies[1:3], w_copies[3:5])[cb]:
            c.start()
        if cb:
            conv_out(cb - 1)
        conv_in(cb)
        lax.fori_loop(0, L // 8, spectra_product, 0)
    conv_out(NCB - 1)

    def rows(i, off=0):
        return pl.ds(pl.multiple_of(i * TM, TM) + off, TM)

    def gate_ln(j, nbuf):
        r0 = pl.multiple_of((j % NB) * TM, TM)
        for s in range(TM // RS):
            r = pl.ds(r0 + s * RS, RS)
            x = xbuf[r, :]
            x = x + _ln(x) * ybuf[r, :]
            xbuf[r, :] = x
            nbuf[s * RS:(s + 1) * RS, :] = _ln(_ln(x)).astype(BF16)

    def w1_job(j, nbuf):
        hb[j // NB, rows(j % NB, 8), :] = _gelu(_dot(nbuf[...], w1[...]))

    def w2_job(t):
        c = D // 4
        l, i = t // NB, t % NB
        r0 = pl.multiple_of(i * TM, TM)
        parts = []
        for g, sh in enumerate((1, -1, 2, -2)):
            win = hb[l, pl.ds(r0, TM + 16), g * c:(g + 1) * c]
            parts.append(pltpu.roll(win, sh % (TM + 16), 0)[8:8 + TM].astype(BF16))
        hsf[...] = _dot(jnp.concatenate(parts, axis=-1), w2[...])

    def ln_u(t, p, on=None):
        r0 = pl.multiple_of((t % NB) * TM + p * PS, PS)
        p0 = pl.multiple_of(p * PS, PS)
        for s in range(PS // 16):
            r = pl.ds(r0 + s * 16, 16)
            x = xbuf[r, :]
            u1 = _ln(x) + hsf[pl.ds(p0 + s * 16, 16), :]
            n2[t % 2, pl.ds(p0 + s * 16, 16), :] = _ln(u1).astype(BF16)
            xbuf[r, :] = x + u1 if on is None else jnp.where(on, x + u1, x)

    w_copies[0].wait()
    xbuf[...] = qbuf[...].astype(F32)
    w_copies[1].wait()

    gate_ln(0, nb0)

    @pl.when(z == 0)
    def _():
        w1_job(0, nb0)
        gate_ln(z + 1, nb1)

    @pl.when(z < 1)
    def _():
        w1_job(1, nb1)
        gate_ln(z + 2, nb0)

    w_copies[2].wait()

    @pl.when(z < 2)
    def _():
        w2_job(0)

    @pl.when(z < 3)
    def _():
        w1_job(2, nb0)
        for p in range(NP):
            ln_u(z, p)

    w_copies[3].wait()
    w_copies[4].wait()

    def out_copy(i):
        return pltpu.make_async_copy(qbuf.at[rows(i), :], o_hbm.at[0, rows(i), :], sem_o.at[i])

    def step(t, _):
        @pl.when(t <= NB)
        def _():
            gate_ln(t + NB - 1, nb0)
            w2_job(t + 1)

        @pl.when(t < NB + 1 + z)
        def _():
            w1_job(t + NB - 1, nb0)

        @pl.when(jnp.logical_and(t > NB, t < 2 * NB - 1))
        def _():
            w2_job(t + 1)

        r = rows(t % NB)

        def fbody(f, _):
            f0 = pl.multiple_of(f * FC, FC)
            g = _gelu(_dot(n2[t % 2], w3[:, pl.ds(f0, FC)])).astype(BF16)
            h2 = _dot(g, w4[pl.ds(f0, FC), :])
            ln_u(t + 1, f, on=t < 2 * NB - 1)
            xn = xbuf[r, :] + h2
            xbuf[r, :] = xn
            qbuf[r, :] = xn.astype(BF16)
            return 0

        lax.fori_loop(0, F // FC, fbody, 0)

        @pl.when(t >= NB)
        def _():
            out_copy(t - NB).start()

        return 0

    lax.fori_loop(0, 2 * NB, step, 0)
    for i in range(NB):
        out_copy(i).wait()


@jax.jit
def pallas_interleave_layers__ssm_conv_h3__mixer_s_mlp__prompt_kernel(
        A_q, A_k, A_v, A_shift_k, A_ssm_k, A_ssm_D, B_x, B_w1, B_w2, B_w3, B_w4):
    fwd, inv = _dft_consts()
    any_spec = pl.BlockSpec(memory_space=pl.ANY)
    vmem_spec = pl.BlockSpec(memory_space=pltpu.VMEM)
    return pl.pallas_call(
        _kernel,
        out_shape=jax.ShapeDtypeStruct((1, S, D), BF16),
        in_specs=[any_spec, any_spec, any_spec, vmem_spec, any_spec, vmem_spec,
                  any_spec, any_spec, any_spec, any_spec, vmem_spec, vmem_spec],
        out_specs=any_spec,
        scratch_shapes=[
            pltpu.VMEM((S, D), F32),
            pltpu.VMEM((S, D), BF16),
            pltpu.VMEM((2, S + 16, D), F32),
            pltpu.VMEM((S, D), F32),
            pltpu.VMEM((D, D), BF16),
            pltpu.VMEM((D, D), BF16),
            pltpu.VMEM((D, F), BF16),
            pltpu.VMEM((F, D), BF16),
            pltpu.VMEM((NCB, S, CB), BF16),
            pltpu.VMEM((NCB, S, CB), BF16),
            pltpu.VMEM((NCB, CB, S), BF16),
            pltpu.VMEM((NC, L, 8 * CB), F32),
            pltpu.SMEM((1,), jnp.int32),
            pltpu.VMEM((2, TM, D), BF16),
            pltpu.VMEM((TM, D), BF16),
            pltpu.VMEM((TM, D), BF16),
            pltpu.VMEM((TM, D), F32),
            pltpu.SemaphoreType.DMA((NCB + 1, 3)),
            pltpu.SemaphoreType.DMA((5,)),
            pltpu.SemaphoreType.DMA((NB,)),
        ],
        compiler_params=pltpu.CompilerParams(vmem_limit_bytes=127 * 1024 * 1024),
    )(A_q, A_k, A_v, A_shift_k.T, A_ssm_k, A_ssm_D, B_w1, B_w2, B_w3, B_w4, fwd, inv)
```
